```python
import jax
import jax.numpy as jnp

def _softmax(x, axis=-1):
    return jax.nn.softmax(x, axis=axis)
def _gelu(x):
    return jax.nn.gelu(x, approximate=True)
def _silu(x):
    return jax.nn.silu(x)
def _sigmoid(x):
    return jax.nn.sigmoid(x)
def _layernorm(x, axis=-1, eps=1e-5):
    m = jnp.mean(x, axis=axis, keepdims=True)
    v = jnp.var(x, axis=axis, keepdims=True)
    return (x - m) / jnp.sqrt(v + eps)
def _scatter_add(tgt, idx, src, axis=0):
    return tgt.at[idx].add(src)
def _segment_sum(src, seg, n):
    return jax.ops.segment_sum(src, seg, n)
class _Rng:
    def __init__(self, key):
        self._k = key
    def _next(self):
        self._k, sub = jax.random.split(self._k)
        return sub
    def normal(self, shape):
        return jax.random.normal(self._next(), shape, dtype=jnp.bfloat16)
    def randint(self, lo, hi, shape):
        return jax.random.randint(self._next(), shape, lo, hi, dtype=jnp.int32)
    def uniform(self, shape, lo=0.0, hi=1.0):
        return jax.random.uniform(self._next(), shape, jnp.bfloat16, lo, hi)
    def permutation(self, n):
        return jax.random.permutation(self._next(), n)


kernel_name = 'parallel_sum__sliding_block_cached__moe_arch_mod__decode'

def setup_inputs():
    _rng = _Rng(jax.random.key(int.from_bytes(__import__("os").urandom(4), "little")))
    _w = (lambda a: (lambda t: t.astype(jnp.bfloat16) if jnp.issubdtype(t.dtype, jnp.floating) else t)(jnp.asarray(a)))
    def _A_setup():
        B, Sq, D = 1, 1, 512
        Hq, Hkv, Sk, Dh = 32, 8, 65536, 128
        assert Hq % Hkv == 0, (Hq, Hkv)
        return {
            "x": _w((lambda *s: _rng.normal(s) * 0.05)(B, Sq, D)),
            "k_cache": _w((lambda *s: _rng.normal(s) * 0.05)(B, Hkv, Sk, Dh)),
            "v_cache": _w((lambda *s: _rng.normal(s) * 0.05)(B, Hkv, Sk, Dh)),
            "wq": _w((lambda *s: _rng.normal(s) * 0.05)(D, Hq * Dh) * (D ** -0.5)),
            "wo": _w((lambda *s: _rng.normal(s) * 0.05)(Hq * Dh, D) * ((Hq * Dh) ** -0.5)),
        }
    _A_in = _A_setup()

    def _B_setup():
        B, S, D, F, C = 1, 1, 512, 1792, 1
        return {
            "x": _w((lambda *s: _rng.normal(s) * 0.05)(B, S, D)),
            "w_r": _w((lambda *s: _rng.normal(s) * 0.05)(D)),
            "w_gate": _w((lambda *s: _rng.normal(s) * 0.05)(D, F)),
            "w_up": _w((lambda *s: _rng.normal(s) * 0.05)(D, F)),
            "w_down": _w((lambda *s: _rng.normal(s) * 0.05)(F, D)),
        }
    _B_in = _B_setup()

    return {
        "A_x": _A_in["x"],
        "A_k_cache": _A_in["k_cache"],
        "A_v_cache": _A_in["v_cache"],
        "A_wq": _A_in["wq"],
        "A_wo": _A_in["wo"],
        "B_x": _B_in["x"],
        "B_w_r": _B_in["w_r"],
        "B_w_gate": _B_in["w_gate"],
        "B_w_up": _B_in["w_up"],
        "B_w_down": _B_in["w_down"],
    }

def reference(A_x, A_k_cache, A_v_cache, A_wq, A_wo, B_x, B_w_r, B_w_gate, B_w_up, B_w_down):
    def _A_ref(x, k_cache, v_cache, wq, wo):
        B, Sq, D = x.shape
        Hq, Dh = 32, 128
        Hkv, Sk = k_cache.shape[1], k_cache.shape[2]
        W = min(4096, max(256, Sk // 4))
        rep = Hq // Hkv
        q = (lambda x, *d: x.transpose(*d))((x @ wq).reshape(B, Sq, Hq, Dh), 0, 2, 1, 3)
        k = jnp.repeat(k_cache[:, :, Sk - W:, :], rep, axis=1)
        v = jnp.repeat(v_cache[:, :, Sk - W:, :], rep, axis=1)
        scores = jnp.einsum("bhqd,bhkd->bhqk", q, k) * (Dh ** -0.5)
        p = _softmax(scores, axis=-1)
        o = jnp.einsum("bhqk,bhkd->bhqd", p, v)
        return (lambda x, *d: x.transpose(*d))(o, 0, 2, 1, 3).reshape(B, Sq, Hq * Dh) @ wo

    def _B_ref(x, w_r, w_gate, w_up, w_down):
        B, S, D = x.shape
        C = 1
        r = x @ w_r
        idx = jnp.argsort(-r, axis=-1)[:, :C]
        idx_e = jnp.repeat(idx.reshape(B, C, 1), D, axis=2)
        x_sel = jnp.take_along_axis(x, idx_e, axis=1)
        g = _silu(x_sel @ w_gate)
        u = x_sel @ w_up
        y = (g * u) @ w_down
        r_sel = _sigmoid(jnp.take_along_axis(r, idx, axis=1))
        y = y * r_sel.reshape(B, C, 1)
        b_off = (jnp.arange(B) * S).reshape(B, 1)
        flat_idx = (idx + b_off).reshape(B * C)
        zero = (x * 0.0).reshape(B * S, D)
        upd = _scatter_add(zero, flat_idx, y.reshape(B * C, D), axis=0)
        return x + upd.reshape(B, S, D)

    x = A_x
    xn = _layernorm(x, axis=-1)
    return x + _A_ref(xn, A_k_cache, A_v_cache, A_wq, A_wo) + _B_ref(xn, B_w_r, B_w_gate, B_w_up, B_w_down)
```

```python
import functools
import jax
import jax.numpy as jnp
from jax import lax
import jax.experimental.pallas as pl
import jax.experimental.pallas.tpu as pltpu

D = 512; HQ = 32; HKV = 8; DH = 128; SK = 65536; F = 1792
W = min(4096, max(256, SK // 4))
REP = HQ // HKV
f32 = jnp.float32; bf16 = jnp.bfloat16


def make_kernel(wd_split=(1024, 512, 256), unroll=False, name="k1", compute=True):
    nd = len(wd_split)

    def loop(n, body):
        if unroll:
            for i in range(n):
                body(i)
        else:
            lax.fori_loop(0, n, lambda i, c: (body(i), c)[1], 0)

    def kernel(x_hbm, k_hbm, v_hbm, wq_hbm, wo_hbm, bx_hbm, wr_hbm, wg_hbm, wu_hbm, wd_hbm, o_ref,
               x_v, wr_v, wq_v, k_v, v_v, wo_v, wg_v, wu_v, wd_v,
               xs, qacc, q_s, p_s, l_s, o_s, acc_s, g_s, u_s, h_s, sems):
        cp_x = pltpu.make_async_copy(x_hbm, x_v, sems.at[0])
        cp_wq = pltpu.make_async_copy(wq_hbm, wq_v, sems.at[1])
        cp_k = pltpu.make_async_copy(k_hbm.at[0, :, pl.ds(SK - W, W), :], k_v, sems.at[2])
        cp_v = pltpu.make_async_copy(v_hbm.at[0, :, pl.ds(SK - W, W), :], v_v, sems.at[3])
        cp_wo = pltpu.make_async_copy(wo_hbm, wo_v, sems.at[4])
        cp_wr = pltpu.make_async_copy(wr_hbm, wr_v, sems.at[5])
        cp_wg = pltpu.make_async_copy(wg_hbm, wg_v, sems.at[6])
        cp_wu = pltpu.make_async_copy(wu_hbm, wu_v, sems.at[7])
        cp_wd = []
        st = 0
        for i, c in enumerate(wd_split):
            cp_wd.append((st, c, pltpu.make_async_copy(wd_hbm.at[pl.ds(st, c), :], wd_v.at[pl.ds(st, c), :], sems.at[8 + i])))
            st += c
        for c in (cp_x, cp_wq, cp_k, cp_v, cp_wo, cp_wr, cp_wg, cp_wu):
            c.start()
        for _, _, c in cp_wd:
            c.start()

        cp_x.wait()
        x = x_v[0].astype(f32)
        mu = jnp.mean(x, axis=-1, keepdims=True)
        xc = x - mu
        var = jnp.mean(xc * xc, axis=-1, keepdims=True)
        xn = (xc / jnp.sqrt(var + 1e-5)).astype(bf16)
        xn32 = xn.astype(f32)
        xn8 = jnp.broadcast_to(xn32, (8, D))
        for kc in range(D // 128):
            xs[kc] = xn8[:, kc * 128:(kc + 1) * 128]

        cp_wq.wait()
        if compute:
            qacc[...] = jnp.zeros(qacc.shape, f32)
            def qbody(kc):
                w = wq_v[pl.ds(pl.multiple_of(kc * 128, 128), 128), :]
                qacc[...] += jnp.dot(xs[kc].astype(bf16), w, preferred_element_type=f32)
            loop(D // 128, qbody)
            row = lax.broadcasted_iota(jnp.int32, (8, DH), 0)
            for h in range(HKV):
                q8 = jnp.zeros((8, DH), f32)
                for j in range(REP):
                    t = h * REP + j
                    q8 = jnp.where(row == j, qacc[:, t * DH:(t + 1) * DH], q8)
                q_s[h] = q8

        cp_k.wait()
        def sbody(h):
            q8 = q_s[h].astype(bf16)
            s = lax.dot_general(q8, k_v[h], (((1,), (1,)), ((), ())), preferred_element_type=f32)
            s = s * (DH ** -0.5)
            m = jnp.max(s, axis=-1, keepdims=True)
            p = jnp.exp(s - m)
            l = jnp.sum(p, axis=-1, keepdims=True)
            p_s[h] = p
            l_s[h] = jnp.broadcast_to(l, (8, DH))
        if compute:
            loop(HKV, sbody)

        cp_v.wait()
        def pvbody(h):
            o = jnp.dot(p_s[h].astype(bf16), v_v[h], preferred_element_type=f32)
            o_s[h] = o / l_s[h]
        if compute:
            loop(HKV, pvbody)

        cp_wo.wait()
        acc_s[...] = jnp.zeros(acc_s.shape, f32)
        def obody(h):
            o = o_s[h]
            row = lax.broadcasted_iota(jnp.int32, (8, DH), 0)
            lhs = jnp.concatenate([jnp.where(row == j, o, 0.0) for j in range(REP)], axis=1).astype(bf16)
            w = wo_v[pl.ds(pl.multiple_of(h * REP * DH, REP * DH), REP * DH), :]
            acc_s[...] += jnp.dot(lhs, w, preferred_element_type=f32)
        if compute:
            loop(HKV, obody)
        attn = jnp.sum(acc_s[...], axis=0, keepdims=True)

        cp_wr.wait()
        wr = wr_v[...].astype(f32).reshape(1, D)
        r = jnp.sum(xn32 * wr, axis=-1, keepdims=True)
        rs = 1.0 / (1.0 + jnp.exp(-r))

        cp_wg.wait()
        g_s[...] = jnp.zeros(g_s.shape, f32)
        def gbody(kc):
            w = wg_v[pl.ds(pl.multiple_of(kc * 128, 128), 128), :]
            g_s[...] += jnp.dot(xs[kc].astype(bf16), w, preferred_element_type=f32)
        if compute:
            loop(D // 128, gbody)
        cp_wu.wait()
        u_s[...] = jnp.zeros(u_s.shape, f32)
        def ubody(kc):
            w = wu_v[pl.ds(pl.multiple_of(kc * 128, 128), 128), :]
            u_s[...] += jnp.dot(xs[kc].astype(bf16), w, preferred_element_type=f32)
        if compute:
            loop(D // 128, ubody)
        g = g_s[...]
        hh = (g / (1.0 + jnp.exp(-g))) * u_s[...]
        hb = hh.astype(bf16)

        y = jnp.zeros((8, D), f32)
        for st, c, cp in cp_wd:
            cp.wait()
            if compute:
                y = y + jnp.dot(hb[:, st:st + c], wd_v[pl.ds(st, c), :], preferred_element_type=f32)
        out = x + attn + (xn32 + y[0:1] * rs)
        o_ref[0] = out.astype(o_ref.dtype)

    anyspec = pl.BlockSpec(memory_space=pl.ANY)

    def fn(*args):
        return pl.pallas_call(
            kernel,
            out_shape=jax.ShapeDtypeStruct((1, 1, D), jnp.bfloat16),
            in_specs=[anyspec] * 10,
            out_specs=pl.BlockSpec(memory_space=pltpu.VMEM),
            scratch_shapes=[
                pltpu.VMEM((1, 1, D), bf16), pltpu.VMEM((D,), bf16),
                pltpu.VMEM((D, HQ * DH), bf16),
                pltpu.VMEM((HKV, W, DH), bf16), pltpu.VMEM((HKV, W, DH), bf16),
                pltpu.VMEM((HQ * DH, D), bf16),
                pltpu.VMEM((D, F), bf16), pltpu.VMEM((D, F), bf16), pltpu.VMEM((F, D), bf16),
                pltpu.VMEM((D // 128, 8, 128), f32),
                pltpu.VMEM((8, HQ * DH), f32),
                pltpu.VMEM((HKV, 8, DH), f32),
                pltpu.VMEM((HKV, 8, W), f32),
                pltpu.VMEM((HKV, 8, DH), f32),
                pltpu.VMEM((HKV, 8, DH), f32),
                pltpu.VMEM((8, D), f32),
                pltpu.VMEM((8, F), f32), pltpu.VMEM((8, F), f32),
                pltpu.VMEM((8, F), f32),
                pltpu.SemaphoreType.DMA((8 + nd,)),
            ],
            compiler_params=pltpu.CompilerParams(vmem_limit_bytes=64 * 1024 * 1024),
            name=name,
        )(*args)
    return fn


_KERNEL = make_kernel(name="attn_moe_decode")


@jax.jit
def pallas_parallel_sum__sliding_block_cached__moe_arch_mod__decode_kernel(
    A_x: jax.Array,
    A_k_cache: jax.Array,
    A_v_cache: jax.Array,
    A_wq: jax.Array,
    A_wo: jax.Array,
    B_x: jax.Array,
    B_w_r: jax.Array,
    B_w_gate: jax.Array,
    B_w_up: jax.Array,
    B_w_down: jax.Array,
):
    return _KERNEL(A_x, A_k_cache, A_v_cache, A_wq, A_wo, B_x, B_w_r, B_w_gate, B_w_up, B_w_down)
```

```python
import jax
import jax.numpy as jnp
from jax import lax
import jax.experimental.pallas as pl
import jax.experimental.pallas.tpu as pltpu

_HQ = 32
_DH = 128
_LANES = 128
_EPS = 1e-5

_WD_MXU_ROWS = (1024, 256)
_WD_VPU_ROWS = (128, 128, 128, 64, 32, 32)

_F32 = jnp.float32
_BF16 = jnp.bfloat16


def _kernel(x_hbm, k_hbm, v_hbm, wq_hbm, wo_hbm, wr_hbm, wg_hbm, wu_hbm, wd_hbm,
            o_hbm,
            x_v, wr_v, wq_v, k_v, v_v, wo_v, wg_v, wu_v, wd_v, o_v,
            xs, qacc, q_s, p_s, l_s, o_s, acc_s, g_s, u_s):
    D = x_hbm.shape[-1]
    F = wg_hbm.shape[-1]
    _, HKV, SK, DH = k_hbm.shape
    W = k_v.shape[1]
    REP = _HQ // HKV
    KC = D // _LANES
    pieces = _WD_MXU_ROWS + _WD_VPU_ROWS
    n_mxu = len(_WD_MXU_ROWS)
    vpu_rows = sum(_WD_VPU_ROWS)

    def for_each(n, body):
        lax.fori_loop(0, n, lambda i, c: (body(i), c)[1], 0)

    def main(sems):
        copy = pltpu.make_async_copy
        cp_wq = copy(wq_hbm, wq_v, sems.at[0])
        cp_x = copy(x_hbm, x_v, sems.at[1])
        cp_k = copy(k_hbm.at[0, :, pl.ds(SK - W, W), :], k_v, sems.at[2])
        cp_v = copy(v_hbm.at[0, :, pl.ds(SK - W, W), :], v_v, sems.at[3])
        cp_wo = copy(wo_hbm, wo_v, sems.at[4])
        cp_wr = copy(wr_hbm, wr_v, sems.at[5])
        cp_wg = copy(wg_hbm, wg_v, sems.at[6])
        cp_wu = copy(wu_hbm, wu_v, sems.at[7])
        cp_out = copy(o_v, o_hbm, sems.at[8])
        cp_wd, st = [], 0
        for i, rows in enumerate(pieces):
            rs_ = pl.ds(st, rows)
            cp_wd.append((st, rows, copy(wd_hbm.at[rs_, :], wd_v.at[rs_, :], sems.at[9 + i])))
            st += rows

        for c in (cp_wq, cp_x, cp_k, cp_v, cp_wo, cp_wr, cp_wg, cp_wu):
            c.start()
        for _, _, c in cp_wd:
            c.start()

        cp_x.wait()
        x = x_v[0].astype(_F32)
        mu = jnp.mean(x, axis=-1, keepdims=True)
        xc = x - mu
        var = jnp.mean(xc * xc, axis=-1, keepdims=True)
        xn = (xc / jnp.sqrt(var + _EPS)).astype(_BF16).astype(_F32)
        xn8 = jnp.broadcast_to(xn, (8, D))
        for kc in range(KC):
            xs[kc] = xn8[:, kc * _LANES:(kc + 1) * _LANES]

        def proj(w_ref, acc_ref):
            acc_ref[...] = jnp.zeros(acc_ref.shape, _F32)

            def body(kc):
                w = w_ref[pl.ds(pl.multiple_of(kc * _LANES, _LANES), _LANES), :]
                acc_ref[...] += jnp.dot(xs[kc].astype(_BF16), w, preferred_element_type=_F32)
            for_each(KC, body)

        cp_wq.wait()
        proj(wq_v, qacc)
        row = lax.broadcasted_iota(jnp.int32, (8, DH), 0)
        for h in range(HKV):
            q8 = jnp.zeros((8, DH), _F32)
            for j in range(REP):
                t = h * REP + j
                q8 = jnp.where(row == j, qacc[:, t * DH:(t + 1) * DH], q8)
            q_s[h] = q8

        cp_k.wait()

        def scores(h):
            s = lax.dot_general(q_s[h].astype(_BF16), k_v[h], (((1,), (1,)), ((), ())),
                                preferred_element_type=_F32)
            s = s * (DH ** -0.5)
            p = jnp.exp(s - jnp.max(s, axis=-1, keepdims=True))
            p_s[h] = p
            l_s[h] = jnp.broadcast_to(jnp.sum(p, axis=-1, keepdims=True), (8, DH))
        for_each(HKV, scores)

        cp_v.wait()

        def pv(h):
            o = jnp.dot(p_s[h].astype(_BF16), v_v[h], preferred_element_type=_F32)
            o_s[h] = o / l_s[h]
        for_each(HKV, pv)

        cp_wo.wait()
        acc_s[...] = jnp.zeros(acc_s.shape, _F32)

        def outproj(h):
            o = o_s[h]
            lhs = jnp.concatenate([jnp.where(row == j, o, 0.0) for j in range(REP)], axis=1)
            w = wo_v[pl.ds(pl.multiple_of(h * REP * DH, REP * DH), REP * DH), :]
            acc_s[...] += jnp.dot(lhs.astype(_BF16), w, preferred_element_type=_F32)
        for_each(HKV, outproj)
        attn = jnp.sum(acc_s[...], axis=0, keepdims=True)

        cp_wr.wait()
        r = jnp.sum(xn * wr_v[...].astype(_F32).reshape(1, D), axis=-1, keepdims=True)
        gate = 1.0 / (1.0 + jnp.exp(-r))

        cp_wg.wait()
        proj(wg_v, g_s)
        cp_wu.wait()
        proj(wu_v, u_s)
        g = g_s[...]
        hid = ((g / (1.0 + jnp.exp(-g))) * u_s[...] * gate).astype(_BF16).astype(_F32)
        hid_row0 = jnp.where(lax.broadcasted_iota(jnp.int32, (8, F), 0) == 0, hid, 0.0).astype(_BF16)
        hcol = jnp.concatenate(
            [jnp.transpose(jnp.broadcast_to(hid[0:1, b:b + _LANES], (_LANES, _LANES)))
             for b in range(F - vpu_rows, F, _LANES)], axis=0)

        base = x + attn + xn
        y = jnp.where(lax.broadcasted_iota(jnp.int32, (8, D), 0) == 0,
                      jnp.broadcast_to(base, (8, D)), 0.0)
        for i, (st, rows, c) in enumerate(cp_wd):
            c.wait()
            w = wd_v[pl.ds(st, rows), :]
            if i < n_mxu:
                y = y + jnp.dot(hid_row0[:, st:st + rows], w, preferred_element_type=_F32)
            else:
                o = st - (F - vpu_rows)
                hc = jnp.concatenate([hcol[o:o + rows, :]] * (D // _LANES), axis=1)
                y = y + jnp.sum((w.astype(_F32) * hc).reshape(rows // 8, 8, D), axis=0)
        o_v[0] = jnp.sum(y, axis=0, keepdims=True).astype(o_v.dtype)
        cp_out.start()
        cp_out.wait()

    pl.run_scoped(main, pltpu.SemaphoreType.DMA((9 + len(pieces),)))


def _call(x, k_cache, v_cache, wq, wo, w_r, w_gate, w_up, w_down, *, interpret=False):
    B, S, D = x.shape
    _, HKV, SK, DH = k_cache.shape
    F = w_gate.shape[1]
    W = min(4096, max(256, SK // 4))
    assert B == 1 and S == 1 and DH == _DH and _HQ % HKV == 0 and _HQ // HKV <= 8
    assert D % _LANES == 0 and sum(_WD_MXU_ROWS) + sum(_WD_VPU_ROWS) == F
    assert sum(_WD_VPU_ROWS) % _LANES == 0 and sum(_WD_MXU_ROWS) % _LANES == 0

    hbm = pl.BlockSpec(memory_space=pl.ANY)
    return pl.pallas_call(
        _kernel,
        out_shape=jax.ShapeDtypeStruct((B, S, D), x.dtype),
        in_specs=[hbm] * 9,
        out_specs=hbm,
        scratch_shapes=[
            pltpu.VMEM((B, S, D), x.dtype),
            pltpu.VMEM((D,), w_r.dtype),
            pltpu.VMEM(wq.shape, wq.dtype),
            pltpu.VMEM((HKV, W, DH), k_cache.dtype),
            pltpu.VMEM((HKV, W, DH), v_cache.dtype),
            pltpu.VMEM(wo.shape, wo.dtype),
            pltpu.VMEM(w_gate.shape, w_gate.dtype),
            pltpu.VMEM(w_up.shape, w_up.dtype),
            pltpu.VMEM(w_down.shape, w_down.dtype),
            pltpu.VMEM((B, S, D), x.dtype),
            pltpu.VMEM((D // _LANES, 8, _LANES), _F32),
            pltpu.VMEM((8, _HQ * DH), _F32),
            pltpu.VMEM((HKV, 8, DH), _F32),
            pltpu.VMEM((HKV, 8, W), _F32),
            pltpu.VMEM((HKV, 8, DH), _F32),
            pltpu.VMEM((HKV, 8, DH), _F32),
            pltpu.VMEM((8, D), _F32),
            pltpu.VMEM((8, F), _F32),
            pltpu.VMEM((8, F), _F32),
        ],
        compiler_params=pltpu.CompilerParams(vmem_limit_bytes=64 * 1024 * 1024),
        name="attn_moe_decode",
        interpret=interpret,
    )(x, k_cache, v_cache, wq, wo, w_r, w_gate, w_up, w_down)


@jax.jit
def pallas_parallel_sum__sliding_block_cached__moe_arch_mod__decode_kernel(
    A_x: jax.Array,
    A_k_cache: jax.Array,
    A_v_cache: jax.Array,
    A_wq: jax.Array,
    A_wo: jax.Array,
    B_x: jax.Array,
    B_w_r: jax.Array,
    B_w_gate: jax.Array,
    B_w_up: jax.Array,
    B_w_down: jax.Array,
):
    del B_x
    return _call(A_x, A_k_cache, A_v_cache, A_wq, A_wo, B_w_r, B_w_gate, B_w_up, B_w_down)
```

```python
import jax
import jax.numpy as jnp
from jax import lax
import jax.experimental.pallas as pl
import jax.experimental.pallas.tpu as pltpu

_HQ = 32
_DH = 128
_LANES = 128
_EPS = 1e-5

_BLOCK = 32
_WD_MXU_ROWS = (1024, 256)
_WD_VPU_ROWS = (128, 128, 128, 64, 32, 32)
_WO_ORDER = (0, 1, 2, 5, 6, 7, 3, 4)

_F32 = jnp.float32
_BF16 = jnp.bfloat16


def _kernel(x_hbm, k_hbm, v_hbm, wq_hbm, wo_hbm, wr_hbm, wg_hbm, wu_hbm, wd_hbm,
            o_hbm,
            x_v, wr_v, wq_v, k_v, v_v, wo_v, wg_v, wu_v, wd_v, o_v,
            xs, qacc, q_s, o_s, acc_s, g_s, u_s, hrow_s, hcol_s):
    D = x_hbm.shape[-1]
    F = wg_hbm.shape[-1]
    _, HKV, SK, DH = k_hbm.shape
    W = k_v.shape[1]
    REP = _HQ // HKV
    KC = D // _LANES
    GR = REP * DH
    B = _BLOCK
    chunks = _WD_MXU_ROWS + _WD_VPU_ROWS
    vpu_rows = sum(_WD_VPU_ROWS)
    S_X, S_WR, S_OUT, S_WQ, S_WG, S_WU = range(6)
    S_K = 6
    S_V = S_K + HKV
    S_WO = S_V + HKV
    S_WD = S_WO + HKV

    def for_each(n, body):
        lax.fori_loop(0, n, lambda i, c: (body(i), c)[1], 0)

    def main(sems):
        copy = pltpu.make_async_copy

        def wq_piece(t, j):
            rows = pl.ds(t * (D // 2) + (j // 2) * 8, 8)
            cols = pl.ds((j % 2) * (_HQ * DH // 2), _HQ * DH // 2)
            return copy(wq_hbm.at[rows, cols], wq_v.at[rows, cols], sems.at[S_WQ])

        def wg_piece(j):
            rows = pl.ds(j * 8, 8)
            return copy(wg_hbm.at[rows, :], wg_v.at[rows, :], sems.at[S_WG])

        def wu_piece(j):
            rows = pl.ds(j * 8, 8)
            return copy(wu_hbm.at[rows, :], wu_v.at[rows, :], sems.at[S_WU])

        kv_rows = W // B

        def k_piece(h, i):
            return copy(k_hbm.at[0, h, pl.ds(SK - W + i * kv_rows, kv_rows), :],
                        k_v.at[h, pl.ds(i * kv_rows, kv_rows), :], sems.at[S_K + h])

        def v_piece(h, i):
            return copy(v_hbm.at[0, h, pl.ds(SK - W + i * kv_rows, kv_rows), :],
                        v_v.at[h, pl.ds(i * kv_rows, kv_rows), :], sems.at[S_V + h])

        def wo_piece(e):
            rows = pl.ds(e * 32, 32)
            return copy(wo_hbm.at[rows, :], wo_v.at[rows, :], sems.at[S_WO + (e * 32) // GR])

        wd_pieces, st = [], 0
        for c, rows in enumerate(chunks):
            step = 32 if rows >= 128 else 16
            wd_pieces += [(st + r, step, c) for r in range(0, rows, step)]
            st += rows

        def wd_piece(n):
            r, rows, c = wd_pieces[n]
            return copy(wd_hbm.at[pl.ds(r, rows), :], wd_v.at[pl.ds(r, rows), :], sems.at[S_WD + c])

        n_wo = _HQ * DH // 32
        n_a = (n_wo + len(wd_pieces) - B) // 2
        assert 2 * n_a == n_wo + len(wd_pieces) - B and 2 * B <= n_a <= n_wo

        def tail_b(n):
            return wo_piece(n_a + n) if n_a + n < n_wo else wd_piece(n - (n_wo - n_a))

        def issue(a, b, n=B):
            for i in range(n):
                a(i).start(priority=0)
                b(i).start(priority=1)

        cp_x = copy(x_hbm, x_v, sems.at[S_X])
        cp_wr = copy(wr_hbm, wr_v, sems.at[S_WR])
        cp_x.start(priority=0)
        cp_wr.start(priority=1)
        for j in range(B):
            wq_piece(1, j).start(priority=1)
        issue(lambda j: wq_piece(0, j), lambda j: wq_piece(1, B + j))
        issue(lambda j: wq_piece(0, B + j), wu_piece)

        cp_x.wait()
        x = x_v[0].astype(_F32)
        mu = jnp.mean(x, axis=-1, keepdims=True)
        xc = x - mu
        var = jnp.mean(xc * xc, axis=-1, keepdims=True)
        xn = (xc / jnp.sqrt(var + _EPS)).astype(_BF16).astype(_F32)
        xn8 = jnp.broadcast_to(xn, (8, D))
        for kc in range(KC):
            xs[kc] = xn8[:, kc * _LANES:(kc + 1) * _LANES]
        cp_wr.wait()
        r = jnp.sum(xn * wr_v[...].astype(_F32).reshape(1, D), axis=-1, keepdims=True)
        gate = 1.0 / (1.0 + jnp.exp(-r))

        def proj(w_ref, acc_ref):
            acc_ref[...] = jnp.zeros(acc_ref.shape, _F32)

            def body(kc):
                w = w_ref[pl.ds(pl.multiple_of(kc * _LANES, _LANES), _LANES), :]
                acc_ref[...] += jnp.dot(xs[kc].astype(_BF16), w, preferred_element_type=_F32)
            for_each(KC, body)

        issue(wg_piece, lambda j: wu_piece(B + j))

        copy(wq_hbm, wq_v, sems.at[S_WQ]).wait()
        proj(wq_v, qacc)
        row = lax.broadcasted_iota(jnp.int32, (8, DH), 0)
        for h in range(HKV):
            q8 = jnp.zeros((8, DH), _F32)
            for j in range(REP):
                t = h * REP + j
                q8 = jnp.where(row == j, qacc[:, t * DH:(t + 1) * DH], q8)
            q_s[h] = q8

        issue(lambda j: wg_piece(B + j), lambda i: v_piece(0, i))
        issue(lambda i: k_piece(0, i), lambda i: v_piece(1, i))

        copy(wg_hbm, wg_v, sems.at[S_WG]).wait()
        proj(wg_v, g_s)

        def hidden():
            copy(wu_hbm, wu_v, sems.at[S_WU]).wait()
            proj(wu_v, u_s)
            g = g_s[...]
            hid = ((g / (1.0 + jnp.exp(-g))) * u_s[...] * gate).astype(_BF16).astype(_F32)
            hrow_s[...] = jnp.where(lax.broadcasted_iota(jnp.int32, (8, F), 0) == 0, hid, 0.0)
            for b in range(vpu_rows // _LANES):
                c0 = F - vpu_rows + b * _LANES
                hcol_s[b * _LANES:(b + 1) * _LANES, :] = jnp.transpose(
                    jnp.broadcast_to(hid[0:1, c0:c0 + _LANES], (_LANES, _LANES)))

        def attend(h):
            copy(k_hbm.at[0, h, pl.ds(SK - W, W), :], k_v.at[h], sems.at[S_K + h]).wait()
            s = lax.dot_general(q_s[h].astype(_BF16), k_v[h], (((1,), (1,)), ((), ())),
                                preferred_element_type=_F32)
            s = s * (DH ** -0.5)
            p = jnp.exp(s - jnp.max(s, axis=-1, keepdims=True))
            l = jnp.sum(p, axis=-1, keepdims=True)
            copy(v_hbm.at[0, h, pl.ds(SK - W, W), :], v_v.at[h], sems.at[S_V + h]).wait()
            o = jnp.dot(p.astype(_BF16), v_v[h], preferred_element_type=_F32)
            o_s[h] = o / l

        def step(h):
            @pl.when(h < HKV - 2)
            def _():
                issue(lambda i: k_piece(h + 1, i), lambda i: v_piece(h + 2, i))

            @pl.when(h == HKV - 2)
            def _():
                issue(lambda i: k_piece(HKV - 1, i), tail_b)

            @pl.when(h == HKV - 1)
            def _():
                issue(wo_piece, lambda i: tail_b(B + i))

            @pl.when(h == 0)
            def _():
                hidden()

            attend(h)

        for_each(HKV, step)
        issue(lambda i: wo_piece(B + i), lambda i: tail_b(2 * B + i), n_a - B)

        acc_s[...] = jnp.zeros(acc_s.shape, _F32)

        def outproj(t):
            h = t
            for tt, hh in enumerate(_WO_ORDER):
                if tt != hh:
                    h = jnp.where(t == tt, hh, h)
            rows = pl.ds(pl.multiple_of(h * GR, GR), GR)
            copy(wo_hbm.at[rows, :], wo_v.at[rows, :], sems.at[S_WO + h]).wait()
            o = o_s[h]
            lhs = jnp.concatenate([jnp.where(row == j, o, 0.0) for j in range(REP)], axis=1)
            acc_s[...] += jnp.dot(lhs.astype(_BF16), wo_v[rows, :], preferred_element_type=_F32)
        for_each(HKV, outproj)
        attn = jnp.sum(acc_s[...], axis=0, keepdims=True)

        base = x + attn + xn
        y = jnp.where(lax.broadcasted_iota(jnp.int32, (8, D), 0) == 0,
                      jnp.broadcast_to(base, (8, D)), 0.0)
        st = 0
        for c, rows in enumerate(chunks):
            rs = pl.ds(st, rows)
            copy(wd_hbm.at[rs, :], wd_v.at[rs, :], sems.at[S_WD + c]).wait()
            w = wd_v[rs, :]
            if c < len(_WD_MXU_ROWS):
                y = y + jnp.dot(hrow_s[:, st:st + rows].astype(_BF16), w, preferred_element_type=_F32)
            else:
                o = st - (F - vpu_rows)
                hc = jnp.concatenate([hcol_s[o:o + rows, :]] * (D // _LANES), axis=1)
                y = y + jnp.sum((w.astype(_F32) * hc).reshape(rows // 8, 8, D), axis=0)
            st += rows
        o_v[0] = jnp.sum(y, axis=0, keepdims=True).astype(o_v.dtype)
        cp_out = copy(o_v, o_hbm, sems.at[S_OUT])
        cp_out.start()
        cp_out.wait()

    pl.run_scoped(main, pltpu.SemaphoreType.DMA((S_WD + len(chunks),)))


@jax.jit
def pallas_parallel_sum__sliding_block_cached__moe_arch_mod__decode_kernel(
    A_x: jax.Array,
    A_k_cache: jax.Array,
    A_v_cache: jax.Array,
    A_wq: jax.Array,
    A_wo: jax.Array,
    B_x: jax.Array,
    B_w_r: jax.Array,
    B_w_gate: jax.Array,
    B_w_up: jax.Array,
    B_w_down: jax.Array,
):
    del B_x
    B, S, D = A_x.shape
    _, HKV, SK, DH = A_k_cache.shape
    F = B_w_gate.shape[1]
    W = min(4096, max(256, SK // 4))
    assert (B, S, D, HKV, DH, W, F) == (1, 1, 512, 8, _DH, 4096, 1792)
    assert sum(_WD_MXU_ROWS) + sum(_WD_VPU_ROWS) == F and sum(_WD_VPU_ROWS) % _LANES == 0

    hbm = pl.BlockSpec(memory_space=pl.ANY)
    return pl.pallas_call(
        _kernel,
        out_shape=jax.ShapeDtypeStruct((B, S, D), A_x.dtype),
        in_specs=[hbm] * 9,
        out_specs=hbm,
        scratch_shapes=[
            pltpu.VMEM((B, S, D), A_x.dtype),
            pltpu.VMEM((D,), B_w_r.dtype),
            pltpu.VMEM(A_wq.shape, A_wq.dtype),
            pltpu.VMEM((HKV, W, DH), A_k_cache.dtype),
            pltpu.VMEM((HKV, W, DH), A_v_cache.dtype),
            pltpu.VMEM(A_wo.shape, A_wo.dtype),
            pltpu.VMEM(B_w_gate.shape, B_w_gate.dtype),
            pltpu.VMEM(B_w_up.shape, B_w_up.dtype),
            pltpu.VMEM(B_w_down.shape, B_w_down.dtype),
            pltpu.VMEM((B, S, D), A_x.dtype),
            pltpu.VMEM((D // _LANES, 8, _LANES), _F32),
            pltpu.VMEM((8, _HQ * DH), _F32),
            pltpu.VMEM((HKV, 8, DH), _F32),
            pltpu.VMEM((HKV, 8, DH), _F32),
            pltpu.VMEM((8, D), _F32),
            pltpu.VMEM((8, F), _F32),
            pltpu.VMEM((8, F), _F32),
            pltpu.VMEM((8, F), _F32),
            pltpu.VMEM((sum(_WD_VPU_ROWS), _LANES), _F32),
        ],
        compiler_params=pltpu.CompilerParams(vmem_limit_bytes=64 * 1024 * 1024),
        name="attn_moe_decode",
    )(A_x, A_k_cache, A_v_cache, A_wq, A_wo, B_w_r, B_w_gate, B_w_up, B_w_down)
```

```python
import jax
import jax.numpy as jnp
from jax import lax
import jax.experimental.pallas as pl
import jax.experimental.pallas.tpu as pltpu

_HQ = 32
_DH = 128
_LANES = 128
_EPS = 1e-5

_BLOCK = 32
_WD_MXU_ROWS = (1280,)
_WD_VPU_ROWS = (128, 128, 128, 64, 32, 16, 16)
_WO_ORDER = (5, 6, 7, 0, 1, 2, 3, 4)
_HEAD_GROUP = 4
_WQ_REGIONS = 4
_GU_REGIONS = 2
_WO_REGIONS = (0, 0)
_WD_REGIONS = 2

_F32 = jnp.float32
_BF16 = jnp.bfloat16


def _kernel(x_hbm, k_hbm, v_hbm, wq_hbm, wo_hbm, wr_hbm, wg_hbm, wu_hbm, wd_hbm,
            o_hbm,
            x_v, wr_v, wq_v, k_v, v_v, wo_v, wg_v, wu_v, wd_v, o_v,
            xs, qacc, q_s, o_s, acc_s, g_s, u_s, hrow_s, hcol_s):
    D = x_hbm.shape[-1]
    F = wg_hbm.shape[-1]
    _, HKV, SK, DH = k_hbm.shape
    W = k_v.shape[1]
    REP = _HQ // HKV
    KC = D // _LANES
    GR = REP * DH
    B = _BLOCK
    chunks = _WD_MXU_ROWS + _WD_VPU_ROWS
    vpu_rows = sum(_WD_VPU_ROWS)
    S_X, S_WR, S_OUT, S_WQ, S_WG, S_WU = range(6)
    S_K = 6
    S_V = S_K + HKV
    S_WO = S_V + HKV
    S_WD = S_WO + HKV

    def for_each(n, body):
        lax.fori_loop(0, n, lambda i, c: (body(i), c)[1], 0)

    def main(sems):
        copy = pltpu.make_async_copy

        def spread(n, regions):
            m = n // regions
            return [r * m + i for i in range(m) for r in range(regions)] + list(range(m * regions, n))

        wq_order = spread(2 * B, _WQ_REGIONS)
        gu_order = spread(2 * B, _GU_REGIONS)

        def wq_piece(t, j):
            j = wq_order[j]
            rows = pl.ds(t * (D // 2) + (j // 2) * 8, 8)
            cols = pl.ds((j % 2) * (_HQ * DH // 2), _HQ * DH // 2)
            return copy(wq_hbm.at[rows, cols], wq_v.at[rows, cols], sems.at[S_WQ])

        def wg_piece(j):
            rows = pl.ds(gu_order[j] * 8, 8)
            return copy(wg_hbm.at[rows, :], wg_v.at[rows, :], sems.at[S_WG])

        def wu_piece(j):
            rows = pl.ds(gu_order[j] * 8, 8)
            return copy(wu_hbm.at[rows, :], wu_v.at[rows, :], sems.at[S_WU])

        kv_rows = W // B
        HG = _HEAD_GROUP

        def kv_piece(src, dst, sem0, g, j, n):
            h = g * HG + n % HG
            r = (j * (B // HG) + n // HG) * kv_rows
            if not isinstance(r, int):
                r = pl.multiple_of(r, kv_rows)
            return copy(src.at[0, h, pl.ds(SK - W + r, kv_rows), :],
                        dst.at[h, pl.ds(r, kv_rows), :], sems.at[sem0 + h])

        def k_piece(g, j, n):
            return kv_piece(k_hbm, k_v, S_K, g, j, n)

        def v_piece(g, j, n):
            return kv_piece(v_hbm, v_v, S_V, g, j, n)

        def wo_piece(e):
            rows = pl.ds(e * 32, 32)
            return copy(wo_hbm.at[rows, :], wo_v.at[rows, :], sems.at[S_WO + (e * 32) // GR])

        wd_pieces, st = [], 0
        for c, rows in enumerate(chunks):
            step = 32 if rows >= 128 else 16
            cur = [(st + r, step, c) for r in range(0, rows, step)]
            if c == 0:
                cur = [cur[i] for i in spread(len(cur), _WD_REGIONS)]
            wd_pieces += cur
            st += rows

        def wd_piece(n):
            r, rows, c = wd_pieces[n]
            return copy(wd_hbm.at[pl.ds(r, rows), :], wd_v.at[pl.ds(r, rows), :], sems.at[S_WD + c])

        n_wo = _HQ * DH // 32
        per_group = GR // 32
        n_a = (n_wo + len(wd_pieces) - B) // 2
        assert 2 * n_a == n_wo + len(wd_pieces) - B and 2 * B <= n_a <= n_wo
        ga = n_a // per_group
        gb = (n_wo - n_a) // per_group
        wo_a = spread(ga * per_group, _WO_REGIONS[0] or ga) + list(range(ga * per_group, n_a))
        lead_b = n_wo - n_a - gb * per_group
        wo_b = [n_a + e for e in list(range(lead_b)) +
                [lead_b + e for e in spread(gb * per_group, _WO_REGIONS[1] or gb)]]

        def tail_a(n):
            return wo_piece(wo_a[n])

        def tail_b(n):
            return wo_piece(wo_b[n]) if n < len(wo_b) else wd_piece(n - len(wo_b))

        def issue(a, b, n=B):
            for i in range(n):
                a(i).start(priority=0)
                b(i).start(priority=1)

        cp_x = copy(x_hbm, x_v, sems.at[S_X])
        cp_wr = copy(wr_hbm, wr_v, sems.at[S_WR])
        cp_x.start(priority=0)
        cp_wr.start(priority=1)
        for j in range(B):
            wq_piece(1, j).start(priority=1)
        issue(lambda j: wq_piece(0, j), lambda j: wq_piece(1, B + j))
        issue(lambda j: wq_piece(0, B + j), wu_piece)

        cp_x.wait()
        x = x_v[0].astype(_F32)
        mu = jnp.mean(x, axis=-1, keepdims=True)
        xc = x - mu
        var = jnp.mean(xc * xc, axis=-1, keepdims=True)
        xn = (xc / jnp.sqrt(var + _EPS)).astype(_BF16).astype(_F32)
        xn8 = jnp.broadcast_to(xn, (8, D))
        for kc in range(KC):
            xs[kc] = xn8[:, kc * _LANES:(kc + 1) * _LANES]
        cp_wr.wait()
        r = jnp.sum(xn * wr_v[...].astype(_F32).reshape(1, D), axis=-1, keepdims=True)
        gate = 1.0 / (1.0 + jnp.exp(-r))

        def proj(w_ref, acc_ref):
            acc_ref[...] = jnp.zeros(acc_ref.shape, _F32)

            def body(kc):
                w = w_ref[pl.ds(pl.multiple_of(kc * _LANES, _LANES), _LANES), :]
                acc_ref[...] += jnp.dot(xs[kc].astype(_BF16), w, preferred_element_type=_F32)
            for_each(KC, body)

        issue(wg_piece, lambda j: wu_piece(B + j))

        copy(wq_hbm, wq_v, sems.at[S_WQ]).wait()
        proj(wq_v, qacc)
        row = lax.broadcasted_iota(jnp.int32, (8, DH), 0)
        for h in range(HKV):
            q8 = jnp.zeros((8, DH), _F32)
            for j in range(REP):
                t = h * REP + j
                q8 = jnp.where(row == j, qacc[:, t * DH:(t + 1) * DH], q8)
            q_s[h] = q8

        issue(lambda j: wg_piece(B + j), lambda n: v_piece(0, 0, n))
        issue(lambda n: k_piece(0, 0, n), lambda n: v_piece(0, 1, n))

        copy(wg_hbm, wg_v, sems.at[S_WG]).wait()
        proj(wg_v, g_s)

        def hidden():
            copy(wu_hbm, wu_v, sems.at[S_WU]).wait()
            proj(wu_v, u_s)
            g = g_s[...]
            hid = ((g / (1.0 + jnp.exp(-g))) * u_s[...] * gate).astype(_BF16).astype(_F32)
            hrow_s[...] = jnp.where(lax.broadcasted_iota(jnp.int32, (8, F), 0) == 0, hid, 0.0)
            for b in range(vpu_rows // _LANES):
                c0 = F - vpu_rows + b * _LANES
                hcol_s[b * _LANES:(b + 1) * _LANES, :] = jnp.transpose(
                    jnp.broadcast_to(hid[0:1, c0:c0 + _LANES], (_LANES, _LANES)))

        def attend(h):
            copy(k_hbm.at[0, h, pl.ds(SK - W, W), :], k_v.at[h], sems.at[S_K + h]).wait()
            s = lax.dot_general(q_s[h].astype(_BF16), k_v[h], (((1,), (1,)), ((), ())),
                                preferred_element_type=_F32)
            s = s * (DH ** -0.5)
            p = jnp.exp(s - jnp.max(s, axis=-1, keepdims=True))
            l = jnp.sum(p, axis=-1, keepdims=True)
            copy(v_hbm.at[0, h, pl.ds(SK - W, W), :], v_v.at[h], sems.at[S_V + h]).wait()
            o = jnp.dot(p.astype(_BF16), v_v[h], preferred_element_type=_F32)
            o_s[h] = o / l

        issue(lambda n: k_piece(0, 1, n), lambda n: v_piece(0, 2, n))
        hidden()
        issue(lambda n: k_piece(0, 2, n), lambda n: v_piece(0, 3, n))
        issue(lambda n: k_piece(0, 3, n), lambda n: v_piece(1, 0, n))

        def step(h):
            @pl.when(h < HG - 1)
            def _():
                issue(lambda n: k_piece(1, h, n), lambda n: v_piece(1, h + 1, n))

            @pl.when(h == HG - 1)
            def _():
                issue(lambda n: k_piece(1, HG - 1, n), tail_b)

            @pl.when(h == HG)
            def _():
                issue(tail_a, lambda n: tail_b(B + n))

            @pl.when(h == HG + 2)
            def _():
                issue(lambda n: tail_a(B + n), lambda n: tail_b(2 * B + n))

            attend(h)

        for_each(HKV, step)
        issue(lambda n: tail_a(2 * B + n), lambda n: tail_b(3 * B + n), n_a - 2 * B)

        acc_s[...] = jnp.zeros(acc_s.shape, _F32)

        def outproj(t):
            h = t
            for tt, hh in enumerate(_WO_ORDER):
                if tt != hh:
                    h = jnp.where(t == tt, hh, h)
            rows = pl.ds(pl.multiple_of(h * GR, GR), GR)
            copy(wo_hbm.at[rows, :], wo_v.at[rows, :], sems.at[S_WO + h]).wait()
            o = o_s[h]
            lhs = jnp.concatenate([jnp.where(row == j, o, 0.0) for j in range(REP)], axis=1)
            acc_s[...] += jnp.dot(lhs.astype(_BF16), wo_v[rows, :], preferred_element_type=_F32)
        for_each(HKV, outproj)
        attn = jnp.sum(acc_s[...], axis=0, keepdims=True)

        base = x + attn + xn
        y = jnp.where(lax.broadcasted_iota(jnp.int32, (8, D), 0) == 0,
                      jnp.broadcast_to(base, (8, D)), 0.0)
        st = 0
        for c, rows in enumerate(chunks):
            rs = pl.ds(st, rows)
            copy(wd_hbm.at[rs, :], wd_v.at[rs, :], sems.at[S_WD + c]).wait()
            w = wd_v[rs, :]
            if c < len(_WD_MXU_ROWS):
                y = y + jnp.dot(hrow_s[:, st:st + rows].astype(_BF16), w, preferred_element_type=_F32)
            else:
                o = st - (F - vpu_rows)
                hc = jnp.concatenate([hcol_s[o:o + rows, :]] * (D // _LANES), axis=1)
                y = y + jnp.sum((w.astype(_F32) * hc).reshape(rows // 8, 8, D), axis=0)
            st += rows
        o_v[0] = jnp.sum(y, axis=0, keepdims=True).astype(o_v.dtype)
        cp_out = copy(o_v, o_hbm, sems.at[S_OUT])
        cp_out.start()
        cp_out.wait()

    pl.run_scoped(main, pltpu.SemaphoreType.DMA((S_WD + len(chunks),)))


@jax.jit
def pallas_parallel_sum__sliding_block_cached__moe_arch_mod__decode_kernel(
    A_x: jax.Array,
    A_k_cache: jax.Array,
    A_v_cache: jax.Array,
    A_wq: jax.Array,
    A_wo: jax.Array,
    B_x: jax.Array,
    B_w_r: jax.Array,
    B_w_gate: jax.Array,
    B_w_up: jax.Array,
    B_w_down: jax.Array,
):
    del B_x
    B, S, D = A_x.shape
    _, HKV, SK, DH = A_k_cache.shape
    F = B_w_gate.shape[1]
    W = min(4096, max(256, SK // 4))
    assert (B, S, D, HKV, DH, W, F) == (1, 1, 512, 8, _DH, 4096, 1792) and _HEAD_GROUP == 4
    assert sum(_WD_MXU_ROWS) + sum(_WD_VPU_ROWS) == F and sum(_WD_VPU_ROWS) % _LANES == 0

    hbm = pl.BlockSpec(memory_space=pl.ANY)
    return pl.pallas_call(
        _kernel,
        out_shape=jax.ShapeDtypeStruct((B, S, D), A_x.dtype),
        in_specs=[hbm] * 9,
        out_specs=hbm,
        scratch_shapes=[
            pltpu.VMEM((B, S, D), A_x.dtype),
            pltpu.VMEM((D,), B_w_r.dtype),
            pltpu.VMEM(A_wq.shape, A_wq.dtype),
            pltpu.VMEM((HKV, W, DH), A_k_cache.dtype),
            pltpu.VMEM((HKV, W, DH), A_v_cache.dtype),
            pltpu.VMEM(A_wo.shape, A_wo.dtype),
            pltpu.VMEM(B_w_gate.shape, B_w_gate.dtype),
            pltpu.VMEM(B_w_up.shape, B_w_up.dtype),
            pltpu.VMEM(B_w_down.shape, B_w_down.dtype),
            pltpu.VMEM((B, S, D), A_x.dtype),
            pltpu.VMEM((D // _LANES, 8, _LANES), _F32),
            pltpu.VMEM((8, _HQ * DH), _F32),
            pltpu.VMEM((HKV, 8, DH), _F32),
            pltpu.VMEM((HKV, 8, DH), _F32),
            pltpu.VMEM((8, D), _F32),
            pltpu.VMEM((8, F), _F32),
            pltpu.VMEM((8, F), _F32),
            pltpu.VMEM((8, F), _F32),
            pltpu.VMEM((sum(_WD_VPU_ROWS), _LANES), _F32),
        ],
        compiler_params=pltpu.CompilerParams(vmem_limit_bytes=64 * 1024 * 1024),
        name="attn_moe_decode",
    )(A_x, A_k_cache, A_v_cache, A_wq, A_wo, B_w_r, B_w_gate, B_w_up, B_w_down)
```
